```python
import os as _os
_os.environ.setdefault("JAX_PLATFORMS", "cpu")
import jax
import jax.numpy as jnp

def _softmax(x, axis=-1):
    return jax.nn.softmax(x, axis=axis)
def _gelu(x):
    return jax.nn.gelu(x, approximate=True)
def _silu(x):
    return jax.nn.silu(x)
def _sigmoid(x):
    return jax.nn.sigmoid(x)
def _layernorm(x, axis=-1, eps=1e-5):
    m = jnp.mean(x, axis=axis, keepdims=True)
    v = jnp.var(x, axis=axis, keepdims=True)
    return (x - m) / jnp.sqrt(v + eps)
def _scatter_add(tgt, idx, src, axis=0):
    return tgt.at[idx].add(src)
def _segment_sum(src, seg, n):
    return jax.ops.segment_sum(src, seg, n)
class _Rng:
    def __init__(self, key):
        self._k = key
    def _next(self):
        self._k, sub = jax.random.split(self._k)
        return sub
    def normal(self, shape):
        return jax.random.normal(self._next(), shape, dtype=jnp.bfloat16)
    def randint(self, lo, hi, shape):
        return jax.random.randint(self._next(), shape, lo, hi, dtype=jnp.int32)
    def uniform(self, shape, lo=0.0, hi=1.0):
        return jax.random.uniform(self._next(), shape, jnp.bfloat16, lo, hi)
    def permutation(self, n):
        return jax.random.permutation(self._next(), n)


kernel_name = 'concat_heads__mha_block_cached__mha_block_cached__near_ridge'

def setup_inputs():
    _rng = _Rng(jax.random.key(int.from_bytes(__import__("os").urandom(4), "little")))
    _w = (lambda a: (lambda t: t.astype(jnp.bfloat16) if jnp.issubdtype(t.dtype, jnp.floating) else t)(jnp.asarray(a)))
    def _A_setup():
        B, Sq, D = 16, 80, 512
        H, Sk, Dh = 32, 80, 128
        return {
            "x": _w((lambda *s: _rng.normal(s) * 0.8)(B, Sq, D)),
            "k_cache": _w((lambda *s: _rng.normal(s) * 0.8)(B, H, Sk, Dh)),
            "v_cache": _w((lambda *s: _rng.normal(s) * 0.05)(B, H, Sk, Dh)),
            "wq": _w((lambda *s: _rng.normal(s) * 0.8)(D, H * Dh) * (D ** -0.5)),
            "wo": _w((lambda *s: _rng.normal(s) * 0.05)(H * Dh, D) * ((H * Dh) ** -0.5)),
        }
    _A_in = _A_setup()

    def _B_setup():
        B, Sq, D = 16, 80, 512
        H, Sk, Dh = 32, 80, 128
        return {
            "x": _w((lambda *s: _rng.normal(s) * 0.8)(B, Sq, D)),
            "k_cache": _w((lambda *s: _rng.normal(s) * 0.8)(B, H, Sk, Dh)),
            "v_cache": _w((lambda *s: _rng.normal(s) * 0.05)(B, H, Sk, Dh)),
            "wq": _w((lambda *s: _rng.normal(s) * 0.8)(D, H * Dh) * (D ** -0.5)),
            "wo": _w((lambda *s: _rng.normal(s) * 0.05)(H * Dh, D) * ((H * Dh) ** -0.5)),
        }
    _B_in = _B_setup()

    return {
        "A_x": _A_in["x"],
        "A_k_cache": _A_in["k_cache"],
        "A_v_cache": _A_in["v_cache"],
        "A_wq": _A_in["wq"],
        "A_wo": _A_in["wo"],
        "B_x": _B_in["x"],
        "B_k_cache": _B_in["k_cache"],
        "B_v_cache": _B_in["v_cache"],
        "B_wq": _B_in["wq"],
        "B_wo": _B_in["wo"],
    }

def reference(A_x, A_k_cache, A_v_cache, A_wq, A_wo, B_x, B_k_cache, B_v_cache, B_wq, B_wo):
    def _A_ref(x, k_cache, v_cache, wq, wo):
        B, Sq, D = x.shape
        H, Dh = 32, 128
        q = (lambda x, *d: x.transpose(*d))((x @ wq).reshape(B, Sq, H, Dh), 0, 2, 1, 3)
        scores = jnp.einsum("bhqd,bhkd->bhqk", q, k_cache) * (Dh ** -0.5)
        p = _softmax(scores, axis=-1)
        o = jnp.einsum("bhqk,bhkd->bhqd", p, v_cache)
        return (lambda x, *d: x.transpose(*d))(o, 0, 2, 1, 3).reshape(B, Sq, H * Dh) @ wo

    def _B_ref(x, k_cache, v_cache, wq, wo):
        B, Sq, D = x.shape
        H, Dh = 32, 128
        q = (lambda x, *d: x.transpose(*d))((x @ wq).reshape(B, Sq, H, Dh), 0, 2, 1, 3)
        scores = jnp.einsum("bhqd,bhkd->bhqk", q, k_cache) * (Dh ** -0.5)
        p = _softmax(scores, axis=-1)
        o = jnp.einsum("bhqk,bhkd->bhqd", p, v_cache)
        return (lambda x, *d: x.transpose(*d))(o, 0, 2, 1, 3).reshape(B, Sq, H * Dh) @ wo

    a = _A_ref(A_x, A_k_cache, A_v_cache, A_wq, A_wo)
    b = _B_ref(B_x, B_k_cache, B_v_cache, B_wq, B_wo)
    return jnp.concatenate([a, b], axis=-1)
```

```python
import functools
import jax
import jax.numpy as jnp
import jax.experimental.pallas as pl
import jax.experimental.pallas.tpu as pltpu

B, SQ, D = 16, 80, 512
H, SK, DH = 32, 80, 128
NUNIT, UB = 4, 4
M = UB * SQ
HB = 8
NBLK = 2 * H // HB
GH = 4
SCALE = (DH ** -0.5) * 1.4426950408889634
bf16, f32 = jnp.bfloat16, jnp.float32


def schedule(NU, NH, LKV=560, LQK=350, LVO=350, LA=4, inflight=2, init=2, endres=1):
    DQ = DO = 320
    DK = DV = 80
    stream = [(u, h) for h in range(NH) for u in range(NU)]
    T = len(stream)
    seq, time = [], 0
    qend, kend = {}, {}
    nq = tk = tv = fills = 0
    oq = []
    usable = 2 * T - 4 * NU - endres - init
    while tv < T or nq < T or oq:
        cands = []
        if tv < tk:
            cands.append((kend[tv] + LKV, 0, 'V'))
        pace_ok = tk < T and (fills - init) >= (tk * usable) // T - 1
        if tk < T and tk < nq and (tk - tv) < inflight and pace_ok:
            cands.append((qend[tk] + LQK, 1, 'K'))
        f = None
        hold = tv < T and nq >= T and len(oq) <= endres
        if nq < T and nq - tk < LA:
            f = (time, 2, 'Q')
        elif oq and not hold:
            f = (oq[0][0], 2, 'O')
            if oq[0][0] > time and nq < T and nq - tk < LA + 4:
                f = (time, 2, 'Q')
        elif nq < T and nq - tk < LA + 4:
            f = (time, 2, 'Q')
        if f:
            cands.append(f)
        if not cands:
            if tk < T and tk < nq:
                cands.append((qend[tk] + LQK, 1, 'K'))
            elif nq < T:
                cands.append((time, 2, 'Q'))
            elif oq:
                cands.append((oq[0][0], 2, 'O'))
        ready = [c for c in cands if c[0] <= time]
        if ready:
            c = min(ready, key=lambda c: c[1])
        else:
            c = min(cands, key=lambda c: (c[0], c[1]))
            time = c[0]
        if c[2] == 'V':
            u, h = stream[tv]
            seq.append(('V', u, h)); time += DV
            if h % GH == GH - 1:
                oq.extend((time + LVO, ('O', u, h // GH, n)) for n in range(4))
            tv += 1
        elif c[2] == 'K':
            seq.append(('K',) + stream[tk]); time += DK; kend[tk] = time; tk += 1
        elif c[2] == 'Q':
            seq.append(('Q',) + stream[nq]); time += DQ; qend[nq] = time; nq += 1; fills += 1
        else:
            seq.append(oq.pop(0)[1]); time += DO; fills += 1
    return seq


def parse_seq(text):
    seq = []
    for tok in text.split():
        if tok.startswith('S:'):
            seq.append(('S', int(tok[2:])))
        elif tok.startswith('W:'):
            items = []
            for it in tok[2:].split(','):
                kind, rng = it[0], it[1:]
                lo, hi = (rng.split('-') + [rng])[:2]
                items.append((kind, int(lo), int(hi) + 1))
            seq.append((tok[0], items))
        else:
            seq.append((tok[0],) + tuple(int(v) for v in tok[1:].split('.')))
    return seq


def qk_t(q, k):
    return jax.lax.dot_general(k, q, (((1,), (1,)), ((), ())), preferred_element_type=f32)


def softmax_t(st):
    m = st[0:8]
    for i in range(1, SK // 8):
        m = jnp.maximum(m, st[8 * i:8 * i + 8])
    m = jnp.max(m, axis=0, keepdims=True)
    p = jnp.exp2(st - m)
    l = p[0:8]
    for i in range(1, SK // 8):
        l = l + p[8 * i:8 * i + 8]
    l = jnp.sum(l, axis=0, keepdims=True)
    return (p * pl.reciprocal(l, approx=False)).astype(bf16)


def pv_t(pt, v):
    return jax.lax.dot_general(pt, v, (((0,), (0,)), ((), ())), preferred_element_type=f32)


def make_kernel(first_text, opt):
    loop_seq = schedule(NUNIT, HB, **opt.get('loop', {}))
    first_seq = parse_seq(first_text)
    first_chunks = []
    for t in first_seq:
        if t[0] == 'W':
            first_chunks += t[1]
    seg1 = [('q', 0, HB), ('k', 0, HB // 2), ('v', 0, HB // 2)]
    seg2 = [('k', HB // 2, HB), ('v', HB // 2, HB), ('o', 0, 2)]
    nfirst = len(first_chunks)
    per = len(seg1) + len(seg2)
    X_SEM = nfirst + per * (NBLK - 1)
    n_in_sems = X_SEM + 1
    NOUT = NUNIT - 1 + 4

    def kernel(xa, ka, va, wqa, woa, xb, kb, vb, wqb, wob, out,
               x_v, k_v, v_v, wq_v, wo_v, acc, stage, isem, osem):
        src = {0: dict(x=xa, k=ka, v=va, q=wqa, o=woa), 1: dict(x=xb, k=kb, v=vb, q=wqb, o=wob)}

        def dst_of(kind, lo, hi, c):
            if kind == 'x':
                return x_v.at[c // 4 if isinstance(c, int) else c, pl.ds(lo * M, (hi - lo) * M)]
            if kind == 'q':
                return wq_v.at[c, :, pl.ds(lo * DH, (hi - lo) * DH)]
            if kind == 'o':
                return wo_v.at[c, pl.ds(lo * GH * DH, (hi - lo) * GH * DH)]
            return (k_v if kind == 'k' else v_v).at[c, :, pl.ds(lo, hi - lo)]

        def copy_in(kind, lo, hi, c, sem):
            br, h0 = c // 4, (c % 4) * HB
            s = src[br][kind]
            if kind == 'x':
                s = s.at[pl.ds(lo * M, (hi - lo) * M)]
            elif kind == 'q':
                s = s.at[:, pl.ds((h0 + lo) * DH, (hi - lo) * DH)]
            elif kind == 'o':
                s = s.at[pl.ds((h0 + lo * GH) * DH, (hi - lo) * GH * DH)]
            else:
                s = s.at[:, pl.ds(h0 + lo, hi - lo)]
            return pltpu.make_async_copy(s, dst_of(kind, lo, hi, c), isem.at[sem])

        def wait_in(kind, lo, hi, c, sem):
            d = dst_of(kind, lo, hi, c)
            pltpu.make_async_copy(d, d, isem.at[sem]).wait()

        def out_copy(j, br):
            if j < NUNIT - 1:
                rows, c0, cw = pl.ds(j * M, M), 0, D
            else:
                rows, c0, cw = pl.ds((NUNIT - 1) * M, M), (j - NUNIT + 1) * 128, 128
            col = br * D + c0
            if not isinstance(col, int):
                col = pl.multiple_of(col, 128)
            return pltpu.make_async_copy(stage.at[rows, pl.ds(c0, cw)], out.at[rows, pl.ds(col, cw)], osem.at[j])

        later = []
        nrun = opt.get('nrun', NBLK)
        for c in range(1, nrun):
            if c == 4:
                later.append(('x', 0, NUNIT, c, X_SEM))
            for j, (kind, lo, hi) in enumerate(seg1 + seg2):
                later.append((kind, lo, hi, c, nfirst + (c - 1) * per + j))

        def run_block(seq, c, br, first):
            xs, qs, sts, os_ = {}, {}, {}, {}
            odone = {}
            widx = 0
            nlater = 0
            import contextlib
            segno = [0]
            cm = [jax.named_scope("lseg0") if (opt.get('scopes') and not first) else contextlib.nullcontext()]
            cm[0].__enter__()
            def newscope(name):
                cm[0].__exit__(None, None, None)
                cm[0] = jax.named_scope(name) if opt.get('scopes') else contextlib.nullcontext()
                cm[0].__enter__()
            for task in seq:
                kind = task[0]
                if kind in 'WM':
                    newscope(f"{'f' if first else 'l'}wait{segno[0]}")
                elif kind in 'QKVO' and not getattr(newscope, 'inseg', False):
                    pass
                if kind == 'W':
                    for (kd, lo, hi) in task[1]:
                        wait_in(kd, lo, hi, 0, widx)
                        widx += 1
                    newscope(f"fseg{segno[0]}"); segno[0] += 1
                elif kind == 'S':
                    n = task[1]
                    for args in later[nlater:nlater + n]:
                        copy_in(*args).start()
                    nlater += n
                elif kind == 'M':
                    for j, (kd, lo, hi) in enumerate(seg2):
                        wait_in(kd, lo, hi, c, nfirst + (c - 1) * per + len(seg1) + j)

                    @pl.when(c > 1)
                    def _():
                        for j in range(NOUT):
                            out_copy(j, 0).wait()
                    newscope("lseg1")
                elif kind == 'Q':
                    _, u, h = task
                    if u not in xs:
                        xs[u] = x_v[br, u * M:(u + 1) * M, :]
                    qv = jnp.dot(xs[u], wq_v[c, :, h * DH:(h + 1) * DH], preferred_element_type=f32) * SCALE
                    qs[u, h] = [qv[b * SQ:(b + 1) * SQ].astype(bf16) for b in range(UB)]
                elif kind == 'K':
                    _, u, h = task
                    q = qs.pop((u, h))
                    sts[u, h] = [qk_t(q[b], k_v[c, u * UB + b, h]) for b in range(UB)]
                elif kind == 'V':
                    _, u, h = task
                    st = sts.pop((u, h))
                    os_[u, h] = jnp.concatenate(
                        [pv_t(softmax_t(st[b]), v_v[c, u * UB + b, h]) for b in range(UB)], axis=0).astype(bf16)
                else:
                    _, u, g, n = task
                    rows, cols = slice(u * M, (u + 1) * M), slice(n * 128, (n + 1) * 128)
                    y = None
                    for j in range(GH):
                        h = g * GH + j
                        d = jnp.dot(os_[u, h], wo_v[c, h * DH:(h + 1) * DH, cols], preferred_element_type=f32)
                        y = d if y is None else y + d
                    if g == 0:
                        if not first:
                            y = y + jnp.where(c == 4, 0.0, acc[rows, cols])
                        acc[rows, cols] = y
                    else:
                        y = y + acc[rows, cols]
                        acc[rows, cols] = y
                        if not first:
                            stage[rows, cols] = y.astype(bf16)
                            odone[u] = odone.get(u, 0) + 1
                            if u == NUNIT - 1:
                                out_copy(NUNIT - 1 + n, br).start()
                            elif odone[u] == 4:
                                out_copy(u, br).start()
            if first:
                for args in later[nlater:]:
                    copy_in(*args).start()
            cm[0].__exit__(None, None, None)

        npre = opt.get('npre', nfirst)
        for j, (kd, lo, hi) in enumerate(first_chunks):
            copy_in(kd, lo, hi, 0, j).start()
        run_block(first_seq, 0, 0, True)

        lseq = list(loop_seq)
        mid = next(i for i, t in enumerate(lseq) if (t[0] in 'KV' and t[2] >= HB // 2) or t[0] == 'O')
        lseq.insert(mid, ('M',))

        def body(c, carry):
            br = c // 4
            for j, (kd, lo, hi) in enumerate(seg1):
                wait_in(kd, lo, hi, c, nfirst + (c - 1) * per + j)

            @pl.when(c == 4)
            def _():
                d = x_v.at[1]
                pltpu.make_async_copy(d, d, isem.at[X_SEM]).wait()

            run_block(lseq, c, br, False)
            return carry

        jax.lax.fori_loop(1, nrun, body, 0)
        if nrun > 1:
            for j in range(NOUT):
                if opt.get('scopes'):
                    with jax.named_scope(f"owait{j}"):
                        out_copy(j, 0).wait()
                else:
                    out_copy(j, 0).wait()

    return kernel, n_in_sems, NOUT


FIRST = """W:x0,q0-1 Q0.0 Q0.1 W:x1,x2 Q1.0 Q1.1 Q2.0 Q2.1 W:x3,q2-3 Q3.0 Q3.1 Q0.2 Q1.2 Q2.2 Q3.2 Q0.3 Q1.3
 W:k0-1,v0-1,q4-7 S:8 K0.0 K1.0 Q2.3 Q3.3 V0.0 V1.0 K2.0 K3.0 Q0.4 Q1.4 V2.0 V3.0 K0.1 K1.1 Q2.4 Q3.4 V0.1 V1.1 K2.1 K3.1 Q0.5 Q1.5 V2.1 V3.1 Q2.5 Q3.5
 W:k2-4,v2-4 S:8 K0.2 K1.2 Q0.6 Q1.6 V0.2 V1.2 K2.2 K3.2 Q2.6 Q3.6 V2.2 V3.2 K0.3 K1.3 Q0.7 Q1.7 V0.3 V1.3 K2.3 K3.3 Q2.7 Q3.7 V2.3 V3.3 K0.4 K1.4
 W:o0,k5-7,v5-7,o1 S:8 O0.0.0 O0.0.1 V0.4 V1.4 K2.4 K3.4 O0.0.2 O0.0.3 V2.4 V3.4 K0.5 K1.5 O1.0.0 O1.0.1 V0.5 V1.5 K2.5 K3.5 O1.0.2 O1.0.3 V2.5 V3.5
 K0.6 K1.6 O2.0.0 O2.0.1 V0.6 V1.6 K2.6 K3.6 O2.0.2 O2.0.3 V2.6 V3.6 K0.7 K1.7 O3.0.0 O3.0.1 V0.7 V1.7 K2.7 K3.7 O3.0.2 O3.0.3 V2.7 V3.7
 O0.1.0 O0.1.1 O0.1.2 O0.1.3 O1.1.0 O1.1.1 O1.1.2 O1.1.3 O2.1.0 O2.1.1 O2.1.2 O2.1.3 O3.1.0 O3.1.1 O3.1.2 O3.1.3"""


def build(first_text=FIRST, opt=None):
    opt = opt or {}
    kernel, n_in, n_out = make_kernel(first_text, opt)

    @jax.jit
    def fn(A_x, A_k_cache, A_v_cache, A_wq, A_wo, B_x, B_k_cache, B_v_cache, B_wq, B_wo):
        out = pl.pallas_call(
            kernel,
            in_specs=[pl.BlockSpec(memory_space=pl.ANY)] * 10,
            out_specs=pl.BlockSpec(memory_space=pl.ANY),
            out_shape=jax.ShapeDtypeStruct((B * SQ, 2 * D), bf16),
            scratch_shapes=[
                pltpu.VMEM((2, B * SQ, D), bf16),
                pltpu.VMEM((NBLK, B, HB, SK, DH), bf16),
                pltpu.VMEM((NBLK, B, HB, SK, DH), bf16),
                pltpu.VMEM((NBLK, D, HB * DH), bf16),
                pltpu.VMEM((NBLK, HB * DH, D), bf16),
                pltpu.VMEM((B * SQ, D), f32),
                pltpu.VMEM((B * SQ, D), bf16),
                pltpu.SemaphoreType.DMA((n_in,)),
                pltpu.SemaphoreType.DMA((n_out,)),
            ],
            compiler_params=pltpu.CompilerParams(
                vmem_limit_bytes=110 * 1024 * 1024, shape_invariant_numerics=False,
                disable_semaphore_checks=bool(opt.get('nosem', 1)), disable_bounds_checks=bool(opt.get('nobounds', 1))),
        )(A_x.reshape(B * SQ, D), A_k_cache, A_v_cache, A_wq, A_wo,
          B_x.reshape(B * SQ, D), B_k_cache, B_v_cache, B_wq, B_wo)
        return out.reshape(B, SQ, 2 * D)
    return fn


pallas_concat_heads__mha_block_cached__mha_block_cached__near_ridge_kernel = build()
```

```python
import jax
import jax.numpy as jnp
import jax.experimental.pallas as pl
import jax.experimental.pallas.tpu as pltpu

B, SQ, D = 16, 80, 512
H, SK, DH = 32, 80, 128
NUNIT, UB = 4, 4
M = UB * SQ
HB = 8
HH = HB // 2
NBLK = 2 * H // HB
BPB = NBLK // 2
GH = 4
NSEM_BLK = 3
SCALE = (DH ** -0.5) * 1.4426950408889634
bf16, f32 = jnp.bfloat16, jnp.float32

_FIRST = """
W:x0,q0 Q0.0
W:q1-2 Q0.1 Q0.2
W:q3,x1 Q0.3 Q1.0 Q1.1 Q1.2 Q1.3
W:x2,q4-7,e1 S:14 Q2.0 Q2.1 Q2.2 Q2.3 Q0.4 Q1.4 Q2.4 Q0.5 Q1.5 Q2.5 Q0.6 Q1.6 Q2.6 Q0.7 Q1.7 Q2.7
 E1.0 E1.1 E1.2
W:x3,e2-3,k0-2,v0-2 S:14 K0.0 K0.1 Q3.0 Q3.1 V0.0 V0.1 K0.2 K1.0 Q3.2 E1.3 V0.2 V1.0 K1.1 K1.2 E2.0 E2.1
 V1.1 V1.2 K2.0 K2.1 E2.2 E2.3 V2.0 V2.1 K2.2 K3.0 Q3.3 Q3.4 V2.2 V3.0 K3.1 K3.2 Q3.5 Q3.6 V3.1 V3.2
 Q3.7 E3.0 E3.1 E3.2 E3.3
W:k3,v3,o0,y0-3,e4-7,k4-5,v4-5 S:14 K0.3 K1.3 E4.0 E4.1 V0.3 V1.3 K2.3 K3.3 E4.2 E4.3 V2.3 V3.3
 K0.4 K0.5 E5.0 E5.1 V0.4 V0.5 K1.4 K1.5 E5.2 E5.3 V1.4 V1.5 K2.4 K2.5 O0.0.0 O0.0.1 V2.4 V2.5
 K3.4 K3.5 O0.0.2 O0.0.3 V3.4 V3.5 O1.0.0 O1.0.1 O1.0.2 O1.0.3 O2.0.0 O2.0.1 O2.0.2 O2.0.3
W:k6-7,v6-7,o1 K0.6 K0.7 O3.0.0 O3.0.1 V0.6 V0.7 K1.6 K1.7 O3.0.2 O3.0.3 V1.6 V1.7 K2.6 K2.7 E6.0 E6.1
 V2.6 V2.7 K3.6 K3.7 E6.2 E6.3 V3.6 V3.7 E7.0 E7.1 E7.2 E7.3 O0.1.0 O0.1.1 O0.1.2 O0.1.3
 O1.1.0 O1.1.1 O1.1.2 O1.1.3 O2.1.0 O2.1.1 O2.1.2 O2.1.3 O3.1.0 O3.1.1 O3.1.2 O3.1.3
"""


def _parse(text):
    seq = []
    for tok in text.split():
        if tok.startswith('S:'):
            seq.append(('S', int(tok[2:])))
        elif tok.startswith('W:'):
            items = []
            for it in tok[2:].split(','):
                lo, hi = (it[1:].split('-') + [it[1:]])[:2]
                items.append((it[0], int(lo), int(hi) + 1))
            seq.append(('W', items))
        else:
            seq.append((tok[0],) + tuple(int(v) for v in tok[1:].split('.')))
    return seq


def _loop_schedule(lat_kv=560, lat_vo=350, ahead=6, inflight=3, reserve=1):
    long_t, short_t = M, SQ
    stream = [(u, h) for h in range(HB) for u in range(NUNIT)]
    total = len(stream)
    seq, now = [], 0
    nq, nk, nv, fills = NUNIT, 0, 0, 0
    q_end = {i: -10 ** 9 for i in range(nq)}
    k_end, o_ready = {}, []
    usable = 2 * total - nq - 4 * NUNIT - reserve
    while nv < total or nq < total or o_ready:
        cands = []
        if nv < nk:
            cands.append((k_end[nv] + lat_kv, 0, 'V'))
        paced = nk < total and fills >= (nk * usable) // total - 1
        if nk < total and nk < nq and nk - nv < inflight and paced:
            cands.append((q_end[nk] + lat_vo, 1, 'K'))
        hold = nv < total and nq >= total and len(o_ready) <= reserve
        fill = None
        if nq < total and nq - nk < ahead:
            fill = (now, 2, 'Q')
        elif o_ready and not hold:
            fill = (o_ready[0][0], 2, 'O')
            if o_ready[0][0] > now and nq < total and nq - nk < ahead + 4:
                fill = (now, 2, 'Q')
        elif nq < total and nq - nk < ahead + 4:
            fill = (now, 2, 'Q')
        if fill:
            cands.append(fill)
        if not cands:
            if nk < total and nk < nq:
                cands.append((q_end[nk] + lat_vo, 1, 'K'))
            elif nq < total:
                cands.append((now, 2, 'Q'))
            else:
                cands.append((o_ready[0][0], 2, 'O'))
        ready = [c for c in cands if c[0] <= now]
        if ready:
            pick = min(ready, key=lambda c: c[1])
        else:
            pick = min(cands, key=lambda c: (c[0], c[1]))
            now = pick[0]
        if pick[2] == 'V':
            u, h = stream[nv]
            seq.append(('V', u, h))
            now += short_t
            if h % GH == GH - 1:
                o_ready.extend((now + lat_vo, ('O', u, h // GH, n)) for n in range(D // 128))
            nv += 1
        elif pick[2] == 'K':
            seq.append(('K',) + stream[nk])
            now += short_t
            k_end[nk] = now
            nk += 1
        elif pick[2] == 'Q':
            seq.append(('Q',) + stream[nq])
            now += long_t
            q_end[nq] = now
            nq += 1
            fills += 1
        else:
            seq.append(o_ready.pop(0)[1])
            now += long_t
            fills += 1
    return seq


def _scores_t(q, k):
    return jax.lax.dot_general(k, q, (((1,), (1,)), ((), ())), preferred_element_type=f32)


def _softmax_t(st):
    m = st[0:8]
    for i in range(1, SK // 8):
        m = jnp.maximum(m, st[8 * i:8 * i + 8])
    m = jnp.max(m, axis=0, keepdims=True)
    p = jnp.exp2(st - m)
    l = p[0:8]
    for i in range(1, SK // 8):
        l = l + p[8 * i:8 * i + 8]
    l = jnp.sum(l, axis=0, keepdims=True)
    return (p * pl.reciprocal(l, approx=False)).astype(bf16)


def _weighted_values(pt, v):
    return jax.lax.dot_general(pt, v, (((0,), (0,)), ((), ())), preferred_element_type=f32)


_FIRST_SEQ = _parse(_FIRST)
_LOOP_SEQ = _loop_schedule()
_GROUPS = [t[1] for t in _FIRST_SEQ if t[0] == 'W']
_NGRP = len(_GROUPS)
_N_IN_SEMS = _NGRP + NSEM_BLK * (NBLK - 1)


def _kernel(xa, ka, va, wqa, woa, xb, kb, vb, wqb, wob, out,
            x_v, kv_v, wq_v, wo_v, qpre, acc, stage, isem, osem):
    src = ({'x': xa, 'k': ka, 'v': va, 'q': wqa, 'o': woa},
           {'x': xb, 'k': kb, 'v': vb, 'q': wqb, 'o': wob})

    def expand(kind, lo, hi):
        if kind in 'kv' and lo < HH < hi:
            return [(kind, lo, HH, 0), (kind, HH, hi, 0)]
        if kind == 'e':
            return [('q', 0, 1, c) for c in range(lo, hi)]
        if kind == 'y':
            return [('x', lo, hi, BPB)]
        return [(kind, lo, hi, 0)]

    def copy_in(kind, lo, hi, c, sem):
        br, h0 = c // BPB, (c % BPB) * HB
        s = src[br][kind]
        if kind == 'x':
            s = s.at[pl.ds(lo * M, (hi - lo) * M)]
            d = x_v.at[br, pl.ds(lo * M, (hi - lo) * M)]
        elif kind == 'q':
            s = s.at[:, pl.ds((h0 + lo) * DH, (hi - lo) * DH)]
            d = wq_v.at[c, :, pl.ds(lo * DH, (hi - lo) * DH)]
        elif kind == 'o':
            s = s.at[pl.ds((h0 + lo * GH) * DH, (hi - lo) * GH * DH)]
            d = wo_v.at[c, pl.ds(lo * GH * DH, (hi - lo) * GH * DH)]
        else:
            s = s.at[:, pl.ds(h0 + lo, hi - lo)]
            d = kv_v.at[c, lo // HH, 0 if kind == 'k' else 1, :, pl.ds(lo % HH, hi - lo)]
        return pltpu.make_async_copy(s, d, isem.at[sem])

    def wait_filled(buf, sem):
        pltpu.make_async_copy(buf, buf, sem).wait()

    later = []
    for c in range(1, NBLK):
        s0 = _NGRP + NSEM_BLK * (c - 1)
        later += [('k', 0, HH, c, s0 + 1), ('v', 0, HH, c, s0 + 1), ('q', 1, HB, c, s0),
                  ('k', HH, HB, c, s0 + 1), ('v', HH, HB, c, s0 + 1), ('o', 0, HB // GH, c, s0 + 2)]

    def start_out(rows, c0, cw, br, c):
        @pl.when((c & (BPB - 1)) == BPB - 1)
        def _():
            col = pl.multiple_of(br * D + c0, 128)
            pltpu.make_async_copy(stage.at[br, rows, pl.ds(c0, cw)],
                                  out.at[rows, pl.ds(col, cw)], osem.at[br]).start()

    def run_block(seq, c, br, first):
        xs, qs, scores, outs, n_out = {}, {}, {}, {}, {}
        group = started = 0

        def x_rows(b_idx, key, u):
            if key not in xs:
                xs[key] = x_v[b_idx, u * M:(u + 1) * M, :]
            return xs[key]

        def kv(which, b, h):
            return kv_v[c, h // HH, which, b, h % HH]

        for task in seq:
            kind = task[0]
            if kind == 'W':
                for item in task[1]:
                    for part in expand(*item):
                        copy_in(*part, group).wait()
                group += 1
            elif kind == 'S':
                for args in later[started:started + task[1]]:
                    copy_in(*args).start()
                started += task[1]
            elif kind == 'E':
                _, cc, u = task
                qv = jnp.dot(x_rows(cc // BPB, (cc // BPB, u), u), wq_v[cc, :, 0:DH],
                             preferred_element_type=f32) * SCALE
                for b in range(UB):
                    qpre[cc - 1, u, b * SQ:(b + 1) * SQ, :] = qv[b * SQ:(b + 1) * SQ].astype(bf16)
            elif kind == 'Q':
                _, u, h = task
                qv = jnp.dot(x_rows(br, (0, u) if first else u, u), wq_v[c, :, h * DH:(h + 1) * DH],
                             preferred_element_type=f32) * SCALE
                qs[u, h] = [qv[b * SQ:(b + 1) * SQ].astype(bf16) for b in range(UB)]
            elif kind == 'K':
                _, u, h = task
                if h == 0 and not first:
                    q = [qpre[c - 1, u, b * SQ:(b + 1) * SQ, :] for b in range(UB)]
                else:
                    q = qs.pop((u, h))
                scores[u, h] = [_scores_t(q[b], kv(0, u * UB + b, h)) for b in range(UB)]
            elif kind == 'V':
                _, u, h = task
                st = scores.pop((u, h))
                o = [_weighted_values(_softmax_t(st[b]), kv(1, u * UB + b, h)) for b in range(UB)]
                outs[u, h] = jnp.concatenate(o, axis=0).astype(bf16)
            else:
                _, u, g, n = task
                rows, cols = slice(u * M, (u + 1) * M), slice(n * 128, (n + 1) * 128)
                y = None
                for j in range(GH):
                    h = g * GH + j
                    d = jnp.dot(outs[u, h], wo_v[c, h * DH:(h + 1) * DH, cols], preferred_element_type=f32)
                    y = d if y is None else y + d
                if g == 0:
                    if not first:
                        y = y + jnp.where(c == BPB, 0.0, acc[rows, cols])
                    acc[rows, cols] = y
                else:
                    y = y + acc[rows, cols]
                    acc[rows, cols] = y
                    if not first:
                        stage[br, rows, cols] = y.astype(bf16)
                        n_out[u] = n_out.get(u, 0) + 1
                        if u == NUNIT - 1:
                            start_out(pl.ds(u * M, M), n * 128, 128, br, c)
                        elif n_out[u] == D // 128:
                            start_out(pl.ds(u * M, M), 0, D, br, c)
        if first:
            for args in later[started:]:
                copy_in(*args).start()

    for g, items in enumerate(_GROUPS):
        for item in items:
            for part in expand(*item):
                copy_in(*part, g).start()
    run_block(_FIRST_SEQ, 0, 0, True)

    def body(c, carry):
        br = jax.lax.shift_right_logical(c, 2)
        s0 = _NGRP + NSEM_BLK * (c - 1)
        wait_filled(kv_v.at[c], isem.at[s0 + 1])
        wait_filled(wq_v.at[c, :, pl.ds(DH, (HB - 1) * DH)], isem.at[s0])
        wait_filled(wo_v.at[c], isem.at[s0 + 2])
        run_block(_LOOP_SEQ, c, br, False)
        return carry

    jax.lax.fori_loop(1, NBLK, body, 0)
    for br in range(2):
        wait_filled(out.at[:, pl.ds(br * D, D)], osem.at[br])


@jax.jit
def pallas_concat_heads__mha_block_cached__mha_block_cached__near_ridge_kernel(
    A_x: jax.Array,
    A_k_cache: jax.Array,
    A_v_cache: jax.Array,
    A_wq: jax.Array,
    A_wo: jax.Array,
    B_x: jax.Array,
    B_k_cache: jax.Array,
    B_v_cache: jax.Array,
    B_wq: jax.Array,
    B_wo: jax.Array,
):
    out = pl.pallas_call(
        _kernel,
        in_specs=[pl.BlockSpec(memory_space=pl.ANY)] * 10,
        out_specs=pl.BlockSpec(memory_space=pl.ANY),
        out_shape=jax.ShapeDtypeStruct((B * SQ, 2 * D), bf16),
        scratch_shapes=[
            pltpu.VMEM((2, B * SQ, D), bf16),
            pltpu.VMEM((NBLK, 2, 2, B, HH, SK, DH), bf16),
            pltpu.VMEM((NBLK, D, HB * DH), bf16),
            pltpu.VMEM((NBLK, HB * DH, D), bf16),
            pltpu.VMEM((NBLK - 1, NUNIT, M, DH), bf16),
            pltpu.VMEM((B * SQ, D), f32),
            pltpu.VMEM((2, B * SQ, D), bf16),
            pltpu.SemaphoreType.DMA((_N_IN_SEMS,)),
            pltpu.SemaphoreType.DMA((2,)),
        ],
        compiler_params=pltpu.CompilerParams(
            vmem_limit_bytes=110 * 1024 * 1024,
            shape_invariant_numerics=False,
            disable_semaphore_checks=True,
            disable_bounds_checks=True,
        ),
    )(A_x.reshape(B * SQ, D), A_k_cache, A_v_cache, A_wq, A_wo,
      B_x.reshape(B * SQ, D), B_k_cache, B_v_cache, B_wq, B_wo)
    return out.reshape(B, SQ, 2 * D)
```

```python
import jax
import jax.numpy as jnp
import jax.experimental.pallas as pl
import jax.experimental.pallas.tpu as pltpu

B, SQ, D = 16, 80, 512
H, SK, DH = 32, 80, 128
NUNIT, UB = 4, 4
M = UB * SQ
HB = 8
NBLK = 2 * H // HB
BPB = NBLK // 2
GH = 4
PRE = 4
NT = D // 128
NSEM_BLK = 3
SCALE = (DH ** -0.5) * 1.4426950408889634
bf16, f32 = jnp.bfloat16, jnp.float32


def _prologue_plan():
    units = range(NUNIT)

    def p(tile, us, blocks):
        return [('P', u, tile, c) for c in blocks for u in us]

    def e(blocks):
        return [('E', c, j, u) for c in blocks for j in range(PRE) for u in units]

    return (
        [('W', [('a', 0, 0, 2), ('b', 0, 0, 1)])] + p(0, (0, 1), (0,))
        + [('W', [('a', 0, 2, 4), ('b', 0, 1, 2)])] + p(0, (2, 3), (0,)) + p(0, units, (1,))
        + [('W', [('a', 1, 0, 4), ('b', 1, 0, 2), ('a', 2, 0, 4), ('b', 2, 0, 1)]), ('S', 8)]
        + p(1, units, (0, 1)) + p(2, units, (0,))
        + [('W', [('b', 2, 1, 2), ('a', 3, 0, 4), ('b', 3, 0, 2), ('e', 2, 4)]), ('S', 12)]
        + p(2, units, (1,)) + p(3, units, (0, 1)) + e((2, 3))
        + [('W', [('y',), ('e', 4, 8)]), ('S', 12)] + e((4, 5, 6, 7))
    )


def _block_plan(lat_kv=560, lat_proj=350, ahead=6, inflight=3, reserve=1):
    long_t, short_t = M, SQ
    stream = [(u, h) for h in range(HB) for u in range(NUNIT)]
    total = len(stream)
    seq, now = [], 0
    nq, nk, nv, fills = PRE * NUNIT, 0, 0, 0
    q_end = {i: -10 ** 9 for i in range(nq)}
    k_end, o_ready = {}, []
    usable = 2 * total - nq - NT * NUNIT - reserve
    while nv < total or nq < total or o_ready:
        cands = []
        if nv < nk:
            cands.append((k_end[nv] + lat_kv, 0, 'V'))
        paced = nk < total and fills >= (nk * usable) // total - 1
        if nk < total and nk < nq and nk - nv < inflight and paced:
            cands.append((q_end[nk] + lat_proj, 1, 'K'))
        hold = nv < total and nq >= total and len(o_ready) <= reserve
        fill = None
        if nq < total and nq - nk < ahead:
            fill = (now, 2, 'Q')
        elif o_ready and not hold:
            fill = (o_ready[0][0], 2, 'O')
            if o_ready[0][0] > now and nq < total:
                fill = (now, 2, 'Q')
        elif nq < total:
            fill = (now, 2, 'Q')
        if fill:
            cands.append(fill)
        if not cands:
            if nk < total and nk < nq:
                cands.append((q_end[nk] + lat_proj, 1, 'K'))
            else:
                cands.append((o_ready[0][0], 2, 'O'))
        ready = [c for c in cands if c[0] <= now]
        if ready:
            pick = min(ready, key=lambda c: c[1])
        else:
            pick = min(cands, key=lambda c: (c[0], c[1]))
            now = pick[0]
        if pick[2] == 'V':
            u, h = stream[nv]
            seq.append(('V', u, h))
            now += short_t
            if h % GH == GH - 1:
                o_ready.extend((now + lat_proj, ('O', u, h // GH, n)) for n in range(NT))
            nv += 1
        elif pick[2] == 'K':
            seq.append(('K',) + stream[nk])
            now += short_t
            k_end[nk] = now
            nk += 1
        elif pick[2] == 'Q':
            seq.append(('Q',) + stream[nq])
            now += long_t
            q_end[nq] = now
            nq += 1
            fills += 1
        else:
            seq.append(o_ready.pop(0)[1])
            now += long_t
            fills += 1
    return seq


_PROLOGUE = _prologue_plan()
_BLOCK = _block_plan()
_GROUPS = [t[1] for t in _PROLOGUE if t[0] == 'W']
_NGRP = len(_GROUPS)
_N_IN_SEMS = _NGRP + NSEM_BLK * NBLK


def _scores_t(q, k):
    return jax.lax.dot_general(k, q, (((1,), (1,)), ((), ())), preferred_element_type=f32)


def _attend(st, v):
    m = st[0:8]
    for i in range(1, SK // 8):
        m = jnp.maximum(m, st[8 * i:8 * i + 8])
    m = jnp.max(m, axis=0, keepdims=True)
    p = jnp.exp2(st - m)
    l = p[0:8]
    for i in range(1, SK // 8):
        l = l + p[8 * i:8 * i + 8]
    l = jnp.sum(l, axis=0, keepdims=True)
    r = jnp.transpose(jnp.broadcast_to(pl.reciprocal(l, approx=False), (DH, SQ)))
    o = jax.lax.dot_general(p.astype(bf16), v, (((0,), (0,)), ((), ())), preferred_element_type=f32)
    return o * r


def _kernel(xa, ka, va, wqa, woa, xb, kb, vb, wqb, wob, out,
            x_v, kv_v, wq_v, wo_v, qpre, qacc, acc, stage, isem, osem):
    k_hbm, v_hbm, wq_hbm, wo_hbm = (ka, kb), (va, vb), (wqa, wqb), (woa, wob)

    def copy(src, dst, sem):
        return pltpu.make_async_copy(src, dst, isem.at[sem])

    def wait_filled(buf, sem):
        pltpu.make_async_copy(buf, buf, sem).wait()

    def prologue_copies(item, sem):
        kind = item[0]
        if kind == 'a':
            _, tile, u0, u1 = item
            rows, cols = pl.ds(u0 * M, (u1 - u0) * M), pl.ds(tile * 128, 128)
            return [copy(xa.at[rows, cols], x_v.at[0, rows, cols], sem)]
        if kind == 'b':
            _, tile, c0, c1 = item
            rows = pl.ds(tile * 128, 128)
            return [copy(wqa.at[rows, pl.ds(c * HB * DH, PRE * DH)],
                         wq_v.at[c, rows, pl.ds(0, PRE * DH)], sem) for c in range(c0, c1)]
        if kind == 'y':
            return [copy(xb, x_v.at[1], sem)]
        _, c0, c1 = item
        return [copy(wq_hbm[c // BPB].at[:, pl.ds((c % BPB) * HB * DH, PRE * DH)],
                     wq_v.at[c, :, pl.ds(0, PRE * DH)], sem) for c in range(c0, c1)]

    block_copies = []
    for c in range(NBLK):
        br, h0, s0 = c // BPB, (c % BPB) * HB, _NGRP + NSEM_BLK * c
        rest = (HB - PRE) * DH
        block_copies += [
            copy(k_hbm[br].at[:, pl.ds(h0, HB)], kv_v.at[c, 0], s0),
            copy(v_hbm[br].at[:, pl.ds(h0, HB)], kv_v.at[c, 1], s0),
            copy(wq_hbm[br].at[:, pl.ds((h0 + PRE) * DH, rest)], wq_v.at[c, :, pl.ds(PRE * DH, rest)], s0 + 1),
            copy(wo_hbm[br].at[pl.ds(h0 * DH, HB * DH)], wo_v.at[c], s0 + 2),
        ]

    def store_q(c, j, u, q):
        for b in range(UB):
            qpre[c, j, u, b * SQ:(b + 1) * SQ, :] = q[b * SQ:(b + 1) * SQ].astype(bf16)

    def prologue():
        group = started = 0
        xs = {}
        for task in _PROLOGUE:
            kind = task[0]
            if kind == 'W':
                for item in task[1]:
                    for cp in prologue_copies(item, group):
                        cp.wait()
                group += 1
            elif kind == 'S':
                for cp in block_copies[started:started + task[1]]:
                    cp.start()
                started += task[1]
            elif kind == 'P':
                _, u, tile, c = task
                ks = slice(tile * 128, (tile + 1) * 128)
                d = jnp.dot(x_v[0, u * M:(u + 1) * M, ks], wq_v[c, ks, 0:PRE * DH],
                            preferred_element_type=f32)
                if tile == 0:
                    qacc[c, u] = d
                elif tile < NT - 1:
                    qacc[c, u] += d
                else:
                    q = (qacc[c, u] + d) * SCALE
                    for j in range(PRE):
                        store_q(c, j, u, q[:, j * DH:(j + 1) * DH])
            else:
                _, c, j, u = task
                key = (c // BPB, u)
                if key not in xs:
                    xs[key] = x_v[c // BPB, u * M:(u + 1) * M, :]
                q = jnp.dot(xs[key], wq_v[c, :, j * DH:(j + 1) * DH], preferred_element_type=f32)
                store_q(c, j, u, q * SCALE)
        assert started == len(block_copies)

    def block(c):
        br = jax.lax.shift_right_logical(c, 2)
        pos = c & (BPB - 1)
        s0 = _NGRP + NSEM_BLK * c
        wait_filled(kv_v.at[c], isem.at[s0])
        wait_filled(wq_v.at[c, :, pl.ds(PRE * DH, (HB - PRE) * DH)], isem.at[s0 + 1])
        wait_filled(wo_v.at[c], isem.at[s0 + 2])

        def start_out(u, c0, width):
            @pl.when(pos == BPB - 1)
            def _():
                rows = pl.ds(u * M, M)
                col = pl.multiple_of(br * D + c0, 128)
                pltpu.make_async_copy(stage.at[br, rows, pl.ds(c0, width)],
                                      out.at[rows, pl.ds(col, width)], osem.at[br]).start()

        xs, qs, scores, outs, n_out = {}, {}, {}, {}, {}
        for task in _BLOCK:
            kind = task[0]
            if kind == 'Q':
                _, u, h = task
                if u not in xs:
                    xs[u] = x_v[br, u * M:(u + 1) * M, :]
                q = jnp.dot(xs[u], wq_v[c, :, h * DH:(h + 1) * DH], preferred_element_type=f32) * SCALE
                qs[u, h] = [q[b * SQ:(b + 1) * SQ].astype(bf16) for b in range(UB)]
            elif kind == 'K':
                _, u, h = task
                if h < PRE:
                    q = [qpre[c, h, u, b * SQ:(b + 1) * SQ, :] for b in range(UB)]
                else:
                    q = qs.pop((u, h))
                scores[u, h] = [_scores_t(q[b], kv_v[c, 0, u * UB + b, h]) for b in range(UB)]
            elif kind == 'V':
                _, u, h = task
                st = scores.pop((u, h))
                o = [_attend(st[b], kv_v[c, 1, u * UB + b, h]) for b in range(UB)]
                outs[u, h] = jnp.concatenate(o, axis=0).astype(bf16)
            else:
                _, u, g, n = task
                rows, cols = slice(u * M, (u + 1) * M), slice(n * 128, (n + 1) * 128)
                y = None
                for j in range(GH):
                    h = g * GH + j
                    d = jnp.dot(outs[u, h], wo_v[c, h * DH:(h + 1) * DH, cols], preferred_element_type=f32)
                    y = d if y is None else y + d
                if g == 0:
                    y = y + jnp.where(pos == 0, 0.0, acc[rows, cols])
                    acc[rows, cols] = y
                else:
                    y = y + acc[rows, cols]
                    acc[rows, cols] = y
                    stage[br, rows, cols] = y.astype(bf16)
                    n_out[u] = n_out.get(u, 0) + 1
                    if u == NUNIT - 1:
                        start_out(u, n * 128, 128)
                    elif n_out[u] == NT:
                        start_out(u, 0, D)

    for group, items in enumerate(_GROUPS):
        for item in items:
            for cp in prologue_copies(item, group):
                cp.start()

    def step(i, carry):
        @pl.when(i > 0)
        def _():
            block(i - 1)

        @pl.when(i == 0)
        def _():
            prologue()
        return carry

    jax.lax.fori_loop(0, NBLK + 1, step, 0)
    for br in range(2):
        wait_filled(out.at[:, pl.ds(br * D, D)], osem.at[br])


@jax.jit
def pallas_concat_heads__mha_block_cached__mha_block_cached__near_ridge_kernel(
    A_x: jax.Array,
    A_k_cache: jax.Array,
    A_v_cache: jax.Array,
    A_wq: jax.Array,
    A_wo: jax.Array,
    B_x: jax.Array,
    B_k_cache: jax.Array,
    B_v_cache: jax.Array,
    B_wq: jax.Array,
    B_wo: jax.Array,
):
    out = pl.pallas_call(
        _kernel,
        in_specs=[pl.BlockSpec(memory_space=pl.ANY)] * 10,
        out_specs=pl.BlockSpec(memory_space=pl.ANY),
        out_shape=jax.ShapeDtypeStruct((B * SQ, 2 * D), bf16),
        scratch_shapes=[
            pltpu.VMEM((2, B * SQ, D), bf16),
            pltpu.VMEM((NBLK, 2, B, HB, SK, DH), bf16),
            pltpu.VMEM((NBLK, D, HB * DH), bf16),
            pltpu.VMEM((NBLK, HB * DH, D), bf16),
            pltpu.VMEM((NBLK, PRE, NUNIT, M, DH), bf16),
            pltpu.VMEM((2, NUNIT, M, PRE * DH), f32),
            pltpu.VMEM((B * SQ, D), f32),
            pltpu.VMEM((2, B * SQ, D), bf16),
            pltpu.SemaphoreType.DMA((_N_IN_SEMS,)),
            pltpu.SemaphoreType.DMA((2,)),
        ],
        compiler_params=pltpu.CompilerParams(
            vmem_limit_bytes=115 * 1024 * 1024,
            shape_invariant_numerics=False,
            disable_semaphore_checks=True,
            disable_bounds_checks=True,
        ),
    )(A_x.reshape(B * SQ, D), A_k_cache, A_v_cache, A_wq, A_wo,
      B_x.reshape(B * SQ, D), B_k_cache, B_v_cache, B_wq, B_wo)
    return out.reshape(B, SQ, 2 * D)
```

```python
import jax
import jax.numpy as jnp
import jax.experimental.pallas as pl
import jax.experimental.pallas.tpu as pltpu

B, SQ, D = 16, 80, 512
H, SK, DH = 32, 80, 128
NUNIT, UB = 4, 4
M = UB * SQ
HB = 8
NBLK = 2 * H // HB
BPB = NBLK // 2
GH = 4
PRE = 4
NT = D // 128
NSEM_BLK = 3
SCALE = (DH ** -0.5) * 1.4426950408889634
bf16, f32 = jnp.bfloat16, jnp.float32


def _prologue_plan():
    units = range(NUNIT)

    def p(tile, us, blocks):
        return [('P', u, tile, c) for c in blocks for u in us]

    def e(blocks):
        return [('E', c, j, u) for c in blocks for j in range(PRE) for u in units]

    return (
        [('W', [('a', 0, 0, 2), ('b', 0, 0, 1)])] + p(0, (0, 1), (0,))
        + [('W', [('a', 0, 2, 4), ('b', 0, 1, 2)])] + p(0, (2, 3), (0,)) + p(0, units, (1,))
        + [('W', [('a', 1, 0, 4), ('b', 1, 0, 2), ('a', 2, 0, 4), ('b', 2, 0, 1)]), ('S', 8)]
        + p(1, units, (0, 1)) + p(2, units, (0,))
        + [('W', [('b', 2, 1, 2), ('a', 3, 0, 4), ('b', 3, 0, 2), ('e', 2, 4)]), ('S', 12)]
        + p(2, units, (1,)) + p(3, units, (0, 1)) + e((2, 3))
        + [('W', [('y',), ('e', 4, 8)]), ('S', 12)] + e((4, 5, 6, 7))
    )


def _block_plan(lat_kv=560, lat_proj=350, ahead=6, inflight=3, reserve=1):
    long_t, short_t = M, SQ
    stream = [(u, h) for h in range(HB) for u in range(NUNIT)]
    total = len(stream)
    seq, now = [], 0
    nq, nk, nv, fills = PRE * NUNIT, 0, 0, 0
    q_end = {i: -10 ** 9 for i in range(nq)}
    k_end, o_ready = {}, []
    usable = 2 * total - nq - NT * NUNIT - reserve
    while nv < total or nq < total or o_ready:
        cands = []
        if nv < nk:
            cands.append((k_end[nv] + lat_kv, 0, 'V'))
        paced = nk < total and fills >= (nk * usable) // total - 1
        if nk < total and nk < nq and nk - nv < inflight and paced:
            cands.append((q_end[nk] + lat_proj, 1, 'K'))
        hold = nv < total and nq >= total and len(o_ready) <= reserve
        fill = None
        if nq < total and nq - nk < ahead:
            fill = (now, 2, 'Q')
        elif o_ready and not hold:
            fill = (o_ready[0][0], 2, 'O')
            if o_ready[0][0] > now and nq < total:
                fill = (now, 2, 'Q')
        elif nq < total:
            fill = (now, 2, 'Q')
        if fill:
            cands.append(fill)
        if not cands:
            if nk < total and nk < nq:
                cands.append((q_end[nk] + lat_proj, 1, 'K'))
            else:
                cands.append((o_ready[0][0], 2, 'O'))
        ready = [c for c in cands if c[0] <= now]
        if ready:
            pick = min(ready, key=lambda c: c[1])
        else:
            pick = min(cands, key=lambda c: (c[0], c[1]))
            now = pick[0]
        if pick[2] == 'V':
            u, h = stream[nv]
            seq.append(('V', u, h))
            now += short_t
            if h % GH == GH - 1:
                o_ready.extend((now + lat_proj, ('O', u, h // GH, n)) for n in range(NT))
            nv += 1
        elif pick[2] == 'K':
            seq.append(('K',) + stream[nk])
            now += short_t
            k_end[nk] = now
            nk += 1
        elif pick[2] == 'Q':
            seq.append(('Q',) + stream[nq])
            now += long_t
            q_end[nq] = now
            nq += 1
            fills += 1
        else:
            seq.append(o_ready.pop(0)[1])
            now += long_t
            fills += 1
    return seq


_PROLOGUE = _prologue_plan()
_BLOCK = _block_plan()
_GROUPS = [t[1] for t in _PROLOGUE if t[0] == 'W']
_NGRP = len(_GROUPS)
_N_IN_SEMS = _NGRP + NSEM_BLK * NBLK


def _scores_t(q, k):
    return jax.lax.dot_general(k, q, (((1,), (1,)), ((), ())), preferred_element_type=f32)


def _softmax_t(st):
    m = st[0:8]
    for i in range(1, SK // 8):
        m = jnp.maximum(m, st[8 * i:8 * i + 8])
    m = jnp.max(m, axis=0, keepdims=True)
    p = jnp.exp2(st - m)
    l = p[0:8]
    for i in range(1, SK // 8):
        l = l + p[8 * i:8 * i + 8]
    l = jnp.sum(l, axis=0, keepdims=True)
    r = jnp.transpose(jnp.broadcast_to(pl.reciprocal(l, approx=False), (DH, SQ)))
    return p.astype(bf16), r


def _attend(pr, v):
    p, r = pr
    o = jax.lax.dot_general(p, v, (((0,), (0,)), ((), ())), preferred_element_type=f32)
    return o * r


def _kernel(xa, ka, va, wqa, woa, xb, kb, vb, wqb, wob, out,
            x_v, kv_v, wq_v, wo_v, qpre, qacc, acc, stage, isem, osem):
    k_hbm, v_hbm, wq_hbm, wo_hbm = (ka, kb), (va, vb), (wqa, wqb), (woa, wob)

    def copy(src, dst, sem):
        return pltpu.make_async_copy(src, dst, isem.at[sem])

    def wait_filled(buf, sem):
        pltpu.make_async_copy(buf, buf, sem).wait()

    def prologue_copies(item, sem):
        kind = item[0]
        if kind == 'a':
            _, tile, u0, u1 = item
            rows, cols = pl.ds(u0 * M, (u1 - u0) * M), pl.ds(tile * 128, 128)
            return [copy(xa.at[rows, cols], x_v.at[0, rows, cols], sem)]
        if kind == 'b':
            _, tile, c0, c1 = item
            rows = pl.ds(tile * 128, 128)
            return [copy(wqa.at[rows, pl.ds(c * HB * DH, PRE * DH)],
                         wq_v.at[c, rows, pl.ds(0, PRE * DH)], sem) for c in range(c0, c1)]
        if kind == 'y':
            return [copy(xb, x_v.at[1], sem)]
        _, c0, c1 = item
        return [copy(wq_hbm[c // BPB].at[:, pl.ds((c % BPB) * HB * DH, PRE * DH)],
                     wq_v.at[c, :, pl.ds(0, PRE * DH)], sem) for c in range(c0, c1)]

    block_copies = []
    for c in range(NBLK):
        br, h0, s0 = c // BPB, (c % BPB) * HB, _NGRP + NSEM_BLK * c
        rest = (HB - PRE) * DH
        block_copies += [
            copy(k_hbm[br].at[:, pl.ds(h0, HB)], kv_v.at[c, 0], s0),
            copy(v_hbm[br].at[:, pl.ds(h0, HB)], kv_v.at[c, 1], s0),
            copy(wq_hbm[br].at[:, pl.ds((h0 + PRE) * DH, rest)], wq_v.at[c, :, pl.ds(PRE * DH, rest)], s0 + 1),
            copy(wo_hbm[br].at[pl.ds(h0 * DH, HB * DH)], wo_v.at[c], s0 + 2),
        ]

    def store_q(c, j, u, q):
        for b in range(UB):
            qpre[c, j, u, b * SQ:(b + 1) * SQ, :] = q[b * SQ:(b + 1) * SQ].astype(bf16)

    def prologue():
        group = started = 0
        xs = {}
        for task in _PROLOGUE:
            kind = task[0]
            if kind == 'W':
                for item in task[1]:
                    for cp in prologue_copies(item, group):
                        cp.wait()
                group += 1
            elif kind == 'S':
                for cp in block_copies[started:started + task[1]]:
                    cp.start()
                started += task[1]
            elif kind == 'P':
                _, u, tile, c = task
                ks = slice(tile * 128, (tile + 1) * 128)
                d = jnp.dot(x_v[0, u * M:(u + 1) * M, ks], wq_v[c, ks, 0:PRE * DH],
                            preferred_element_type=f32)
                if tile == 0:
                    qacc[c, u] = d
                elif tile < NT - 1:
                    qacc[c, u] += d
                else:
                    q = (qacc[c, u] + d) * SCALE
                    for j in range(PRE):
                        store_q(c, j, u, q[:, j * DH:(j + 1) * DH])
            else:
                _, c, j, u = task
                key = (c // BPB, u)
                if key not in xs:
                    xs[key] = x_v[c // BPB, u * M:(u + 1) * M, :]
                q = jnp.dot(xs[key], wq_v[c, :, j * DH:(j + 1) * DH], preferred_element_type=f32)
                store_q(c, j, u, q * SCALE)
        assert started == len(block_copies)

    def block(c):
        br = jax.lax.shift_right_logical(c, 2)
        pos = c & (BPB - 1)
        s0 = _NGRP + NSEM_BLK * c
        wait_filled(kv_v.at[c], isem.at[s0])
        wait_filled(wq_v.at[c, :, pl.ds(PRE * DH, (HB - PRE) * DH)], isem.at[s0 + 1])
        wait_filled(wo_v.at[c], isem.at[s0 + 2])

        def start_out(u, c0, width):
            @pl.when(pos == BPB - 1)
            def _():
                rows = pl.ds(u * M, M)
                col = pl.multiple_of(br * D + c0, 128)
                pltpu.make_async_copy(stage.at[br, rows, pl.ds(c0, width)],
                                      out.at[rows, pl.ds(col, width)], osem.at[br]).start()

        xs, qs, scores, outs, n_out = {}, {}, {}, {}, {}
        for task in _BLOCK:
            kind = task[0]
            if kind == 'Q':
                _, u, h = task
                if u not in xs:
                    xs[u] = x_v[br, u * M:(u + 1) * M, :]
                q = jnp.dot(xs[u], wq_v[c, :, h * DH:(h + 1) * DH], preferred_element_type=f32) * SCALE
                qs[u, h] = [q[b * SQ:(b + 1) * SQ].astype(bf16) for b in range(UB)]
            elif kind == 'K':
                _, u, h = task
                if h < PRE:
                    q = [qpre[c, h, u, b * SQ:(b + 1) * SQ, :] for b in range(UB)]
                else:
                    q = qs.pop((u, h))
                scores[u, h] = [_softmax_t(_scores_t(q[b], kv_v[c, 0, u * UB + b, h])) for b in range(UB)]
            elif kind == 'V':
                _, u, h = task
                st = scores.pop((u, h))
                o = [_attend(st[b], kv_v[c, 1, u * UB + b, h]) for b in range(UB)]
                outs[u, h] = jnp.concatenate(o, axis=0).astype(bf16)
            else:
                _, u, g, n = task
                rows, cols = slice(u * M, (u + 1) * M), slice(n * 128, (n + 1) * 128)
                y = None
                for j in range(GH):
                    h = g * GH + j
                    d = jnp.dot(outs[u, h], wo_v[c, h * DH:(h + 1) * DH, cols], preferred_element_type=f32)
                    y = d if y is None else y + d
                if g == 0:
                    y = y + jnp.where(pos == 0, 0.0, acc[rows, cols])
                    acc[rows, cols] = y
                else:
                    y = y + acc[rows, cols]
                    acc[rows, cols] = y
                    stage[br, rows, cols] = y.astype(bf16)
                    n_out[u] = n_out.get(u, 0) + 1
                    if u == NUNIT - 1:
                        start_out(u, n * 128, 128)
                    elif n_out[u] == NT:
                        start_out(u, 0, D)

    for group, items in enumerate(_GROUPS):
        for item in items:
            for cp in prologue_copies(item, group):
                cp.start()

    def step(i, carry):
        @pl.when(i > 0)
        def _():
            block(i - 1)

        @pl.when(i == 0)
        def _():
            prologue()
        return carry

    jax.lax.fori_loop(0, NBLK + 1, step, 0)
    for br in range(2):
        wait_filled(out.at[:, pl.ds(br * D, D)], osem.at[br])


@jax.jit
def pallas_concat_heads__mha_block_cached__mha_block_cached__near_ridge_kernel(
    A_x: jax.Array,
    A_k_cache: jax.Array,
    A_v_cache: jax.Array,
    A_wq: jax.Array,
    A_wo: jax.Array,
    B_x: jax.Array,
    B_k_cache: jax.Array,
    B_v_cache: jax.Array,
    B_wq: jax.Array,
    B_wo: jax.Array,
):
    out = pl.pallas_call(
        _kernel,
        in_specs=[pl.BlockSpec(memory_space=pl.ANY)] * 10,
        out_specs=pl.BlockSpec(memory_space=pl.ANY),
        out_shape=jax.ShapeDtypeStruct((B * SQ, 2 * D), bf16),
        scratch_shapes=[
            pltpu.VMEM((2, B * SQ, D), bf16),
            pltpu.VMEM((NBLK, 2, B, HB, SK, DH), bf16),
            pltpu.VMEM((NBLK, D, HB * DH), bf16),
            pltpu.VMEM((NBLK, HB * DH, D), bf16),
            pltpu.VMEM((NBLK, PRE, NUNIT, M, DH), bf16),
            pltpu.VMEM((2, NUNIT, M, PRE * DH), f32),
            pltpu.VMEM((B * SQ, D), f32),
            pltpu.VMEM((2, B * SQ, D), bf16),
            pltpu.SemaphoreType.DMA((_N_IN_SEMS,)),
            pltpu.SemaphoreType.DMA((2,)),
        ],
        compiler_params=pltpu.CompilerParams(
            vmem_limit_bytes=115 * 1024 * 1024,
            shape_invariant_numerics=False,
            disable_semaphore_checks=True,
            disable_bounds_checks=True,
        ),
    )(A_x.reshape(B * SQ, D), A_k_cache, A_v_cache, A_wq, A_wo,
      B_x.reshape(B * SQ, D), B_k_cache, B_v_cache, B_wq, B_wo)
    return out.reshape(B, SQ, 2 * D)
```
